```python
import os as _os
_os.environ.setdefault("JAX_PLATFORMS", "cpu")
import jax
import jax.numpy as jnp

def _softmax(x, axis=-1):
    return jax.nn.softmax(x, axis=axis)
def _gelu(x):
    return jax.nn.gelu(x, approximate=True)
def _silu(x):
    return jax.nn.silu(x)
def _sigmoid(x):
    return jax.nn.sigmoid(x)
def _layernorm(x, axis=-1, eps=1e-5):
    m = jnp.mean(x, axis=axis, keepdims=True)
    v = jnp.var(x, axis=axis, keepdims=True)
    return (x - m) / jnp.sqrt(v + eps)
def _scatter_add(tgt, idx, src, axis=0):
    return tgt.at[idx].add(src)
def _segment_sum(src, seg, n):
    return jax.ops.segment_sum(src, seg, n)
class _Rng:
    def __init__(self, key):
        self._k = key
    def _next(self):
        self._k, sub = jax.random.split(self._k)
        return sub
    def normal(self, shape):
        return jax.random.normal(self._next(), shape, dtype=jnp.bfloat16)
    def randint(self, lo, hi, shape):
        return jax.random.randint(self._next(), shape, lo, hi, dtype=jnp.int32)
    def uniform(self, shape, lo=0.0, hi=1.0):
        return jax.random.uniform(self._next(), shape, jnp.bfloat16, lo, hi)
    def permutation(self, n):
        return jax.random.permutation(self._next(), n)


kernel_name = 'standalone__linear_kernel_hedgehog__prompt'

def setup_inputs():
    _rng = _Rng(jax.random.key(int.from_bytes(__import__("os").urandom(4), "little")))
    _w = (lambda a: (lambda t: t.astype(jnp.bfloat16) if jnp.issubdtype(t.dtype, jnp.floating) else t)(jnp.asarray(a)))
    B, S, D, H = 1, 2048, 1024, 32
    Dh = D // H
    return {
        "x": _w((lambda *s: _rng.normal(s) * 0.4)(B, S, D)),
        "wqkv": _w((lambda *s: _rng.normal(s) * 0.4)(D, 3 * D)),
        "w_phi": _w((lambda *s: _rng.normal(s) * 0.4)(H, Dh, Dh) * (Dh ** -0.5)),
        "wo": _w((lambda *s: _rng.normal(s) * 0.05)(D, D)),
    }

def reference(x, wqkv, w_phi, wo):
    B, S, D = x.shape
    H = 32; Dh = D // H
    qkv = (lambda x, *d: x.transpose(*d))((x @ wqkv).reshape(B, S, 3, H, Dh), 2, 0, 3, 1, 4)
    q, k, v = qkv[0], qkv[1], qkv[2]
    pq = jnp.einsum("bhsd,hdf->bhsf", q, w_phi)
    pk = jnp.einsum("bhsd,hdf->bhsf", k, w_phi)
    phi_q = jnp.concatenate([_softmax(pq, axis=-1), _softmax(-pq, axis=-1)], axis=-1)
    phi_k = jnp.concatenate([_softmax(pk, axis=-1), _softmax(-pk, axis=-1)], axis=-1)
    kv = jnp.einsum("bhsf,bhsd->bhfd", phi_k, v)
    z  = jnp.einsum("bhsf->bhf", phi_k)
    num = jnp.einsum("bhqf,bhfd->bhqd", phi_q, kv)
    den = jnp.einsum("bhqf,bhf->bhq", phi_q, z)[..., None] + 1e-6
    o = num / den
    return (lambda x, *d: x.transpose(*d))(o, 0, 2, 1, 3).reshape(B, S, D) @ wo
```

```python
import jax
import jax.numpy as jnp
from jax import lax
import jax.experimental.pallas as pl
import jax.experimental.pallas.tpu as pltpu

S, D, H, DH = 2048, 1024, 32, 32
ST = 512
NTILE = S // ST
G = 8
NT_DIMS = (((1,), (1,)), ((), ()))
F32 = jnp.float32
BF16 = jnp.bfloat16


def _dual_softmax_t(p):
    st = p.shape[-1]
    p3 = p.reshape(16, 8, st)
    mx = jnp.max(p3, axis=0)
    mx = jnp.maximum(mx, pltpu.roll(mx, 4, 0))
    mn = jnp.min(p3, axis=0)
    mn = jnp.minimum(mn, pltpu.roll(mn, 4, 0))
    ep = jnp.exp(p3 - mx[None])
    en = jnp.exp(mn[None] - p3)
    sp = jnp.sum(ep, axis=0)
    sp = sp + pltpu.roll(sp, 4, 0)
    sn = jnp.sum(en, axis=0)
    sn = sn + pltpu.roll(sn, 4, 0)
    php = (ep * (1.0 / sp)[None]).reshape(128, st)
    phn = (en * (1.0 / sn)[None]).reshape(128, st)
    return php, phn


def _kernel(x_ref, wqkv_hbm, wphi_hbm, wo_hbm, o_ref,
            wq_buf, wk_buf, wv_buf, wo_buf, wphi_buf, a_buf, wfold, kv_acc, z_acc, lhs2, sems):
    step = pl.program_id(0)

    def cp_wphi():
        return pltpu.make_async_copy(wphi_hbm, wphi_buf, sems.at[0])

    def cp_wk():
        return pltpu.make_async_copy(wqkv_hbm.at[:, pl.ds(D, D)], wk_buf, sems.at[1])

    def cp_wv():
        return pltpu.make_async_copy(wqkv_hbm.at[:, pl.ds(2 * D, D)], wv_buf, sems.at[2])

    def cp_wq():
        return pltpu.make_async_copy(wqkv_hbm.at[:, pl.ds(0, D)], wq_buf, sems.at[3])

    def cp_wo():
        return pltpu.make_async_copy(wo_hbm, wo_buf, sems.at[4])

    def fold(w_buf):
        for g in range(G):
            wfold[128 * g:128 * (g + 1), :] = lax.dot_general(
                a_buf[:, 128 * g:128 * (g + 1)], w_buf[:, 128 * g:128 * (g + 1)],
                NT_DIMS, preferred_element_type=F32).astype(BF16)

    @pl.when(step == 0)
    def _():
        cp_wphi().start()
        cp_wk().start()
        cp_wv().start()
        cp_wq().start()
        cp_wo().start()
        cp_wphi().wait()
        r = lax.broadcasted_iota(jnp.int32, (128, DH), 0)
        c = lax.broadcasted_iota(jnp.int32, (128, DH), 1)
        perm = (r // 4 == c).astype(BF16)
        a = lax.dot_general(perm, wphi_buf[...], NT_DIMS, preferred_element_type=F32)
        r = lax.broadcasted_iota(jnp.int32, (128, D), 0)
        c = lax.broadcasted_iota(jnp.int32, (128, D), 1)
        a_buf[...] = jnp.where((r % 4) == ((c % 128) // 32), a, 0.0).astype(BF16)
        cp_wk().wait()
        fold(wk_buf)
        kv_acc[...] = jnp.zeros_like(kv_acc)
        z_acc[...] = jnp.zeros_like(z_acc)
        cp_wv().wait()

    @pl.when(step < NTILE)
    def _():
        xt = x_ref[...]
        v = jnp.dot(xt, wv_buf[...], preferred_element_type=F32).astype(BF16)
        pt = lax.dot_general(wfold[...], xt, NT_DIMS, preferred_element_type=F32)
        for g in range(G):
            php, phn = _dual_softmax_t(pt[128 * g:128 * (g + 1), :])
            phi = jnp.concatenate([php, phn], axis=0)
            zp = phi[:, 0:128]
            for j in range(1, ST // 128):
                zp = zp + phi[:, 128 * j:128 * (j + 1)]
            z_acc[g] += zp
            kv_acc[g] += jnp.dot(phi.astype(BF16), v[:, 128 * g:128 * (g + 1)],
                                 preferred_element_type=F32)

    @pl.when(step == NTILE)
    def _():
        r = lax.broadcasted_iota(jnp.int32, (128, 256), 0)
        c = lax.broadcasted_iota(jnp.int32, (128, 256), 1)
        kmask = (c % 4) == (r // 32)
        r = lax.broadcasted_iota(jnp.int32, (16, 256), 0)
        c = lax.broadcasted_iota(jnp.int32, (16, 256), 1)
        zmask = (c % 4) == r
        for g in range(G):
            kvt = kv_acc[g].T
            lhs2[g, 0:128, :] = jnp.where(kmask, kvt, 0.0).astype(BF16)
            zr = jnp.sum(z_acc[g].T, axis=0, keepdims=True)
            lhs2[g, 128:144, :] = jnp.where(zmask, jnp.broadcast_to(zr, (16, 256)), 0.0).astype(BF16)
        cp_wq().wait()
        fold(wq_buf)
        cp_wo().wait()

    @pl.when(step >= NTILE)
    def _():
        xt = x_ref[...]
        pt = lax.dot_general(wfold[...], xt, NT_DIMS, preferred_element_type=F32)
        parts = []
        for g in range(G):
            php, phn = _dual_softmax_t(pt[128 * g:128 * (g + 1), :])
            phi = jnp.concatenate([php, phn], axis=0).astype(BF16)
            r = jnp.dot(lhs2[g], phi, preferred_element_type=F32)
            inv = 1.0 / (r[128:136, :] + 1e-6)
            for hl in range(4):
                parts.append(r[32 * hl:32 * (hl + 1), :] * inv[hl:hl + 1, :])
        ot = jnp.concatenate(parts, axis=0)
        o = ot.T.astype(BF16)
        o_ref[...] = jnp.dot(o, wo_buf[...], preferred_element_type=F32).astype(o_ref.dtype)


@jax.jit
def pallas_standalone__linear_kernel_hedgehog__prompt_kernel(
    x: jax.Array,
    wqkv: jax.Array,
    w_phi: jax.Array,
    wo: jax.Array,
):
    x2 = x.reshape(S, D)
    wphi2 = w_phi.reshape(H * DH, DH)
    out = pl.pallas_call(
        _kernel,
        grid=(2 * NTILE,),
        in_specs=[
            pl.BlockSpec((ST, D), lambda i: (i % NTILE, 0)),
            pl.BlockSpec(memory_space=pl.ANY),
            pl.BlockSpec(memory_space=pl.ANY),
            pl.BlockSpec(memory_space=pl.ANY),
        ],
        out_specs=pl.BlockSpec((ST, D), lambda i: (jnp.maximum(i - NTILE, 0), 0)),
        out_shape=jax.ShapeDtypeStruct((S, D), x.dtype),
        scratch_shapes=[
            pltpu.VMEM((D, D), BF16),
            pltpu.VMEM((D, D), BF16),
            pltpu.VMEM((D, D), BF16),
            pltpu.VMEM((D, D), BF16),
            pltpu.VMEM((H * DH, DH), BF16),
            pltpu.VMEM((128, D), BF16),
            pltpu.VMEM((D, D), BF16),
            pltpu.VMEM((G, 256, 128), F32),
            pltpu.VMEM((G, 256, 128), F32),
            pltpu.VMEM((G, 144, 256), BF16),
            pltpu.SemaphoreType.DMA((5,)),
        ],
        compiler_params=pltpu.CompilerParams(
            dimension_semantics=("arbitrary",),
            vmem_limit_bytes=100 * 1024 * 1024,
        ),
    )(x2, wqkv, wphi2, wo)
    return out.reshape(1, S, D)
```

```python
import jax
import jax.numpy as jnp
from jax import lax
import jax.experimental.pallas as pl
import jax.experimental.pallas.tpu as pltpu

S, D, H, DH = 2048, 1024, 32, 32
ST = 512
NTILE = S // ST
G = 8
NP = 16
XR = 256
NXC = S // XR
WC = 4
OC = 4
LOG2E = 1.4426950408889634
NT_DIMS = (((1,), (1,)), ((), ()))
F32 = jnp.float32
BF16 = jnp.bfloat16

SEM_X = 0
SEM_WK = SEM_X + NXC
SEM_WV = SEM_WK + WC
SEM_WPHI = SEM_WV + WC
SEM_WQ = SEM_WPHI + 1
SEM_WO = SEM_WQ + 1
SEM_OUT = SEM_WO + 1
NSEM = SEM_OUT + NTILE * OC


def _red2(x, op):
    x = op(x, pltpu.roll(x, 2, 0))
    return op(x, pltpu.roll(x, 4, 0))


def _dual_softmax_t(p):
    st = p.shape[-1]
    p3 = p.reshape(8, 8, st)
    mx = _red2(jnp.max(p3, axis=0), jnp.maximum)
    mn = _red2(jnp.min(p3, axis=0), jnp.minimum)
    ep = jnp.exp2(p3 - mx[None])
    en = jnp.exp2(mn[None] - p3)
    sp = _red2(jnp.sum(ep, axis=0), jnp.add)
    sn = _red2(jnp.sum(en, axis=0), jnp.add)
    php = ep * (1.0 / sp)[None]
    phn = en * (1.0 / sn)[None]
    return php, phn


def _kernel(x_hbm, wqkv_hbm, wphi_hbm, wo_hbm, o_hbm,
            x_buf, wq_buf, wk_buf, wv_buf, wo_buf, wphi_buf, a_buf, wfk, wvt, wfq,
            kvt_acc, z_acc, lhs2, zb, o_buf, sems):

    def cp_x(i):
        return pltpu.make_async_copy(x_hbm.at[pl.ds(i * XR, XR), :], x_buf.at[pl.ds(i * XR, XR), :],
                                     sems.at[SEM_X + i])

    def cp_wk(c):
        w = D // WC
        return pltpu.make_async_copy(wqkv_hbm.at[:, pl.ds(D + c * w, w)], wk_buf.at[:, pl.ds(c * w, w)],
                                     sems.at[SEM_WK + c])

    def cp_wv(c):
        w = D // WC
        return pltpu.make_async_copy(wqkv_hbm.at[:, pl.ds(2 * D + c * w, w)], wv_buf.at[:, pl.ds(c * w, w)],
                                     sems.at[SEM_WV + c])

    def cp_wphi():
        return pltpu.make_async_copy(wphi_hbm, wphi_buf, sems.at[SEM_WPHI])

    def cp_wq():
        return pltpu.make_async_copy(wqkv_hbm.at[:, pl.ds(0, D)], wq_buf, sems.at[SEM_WQ])

    def cp_wo():
        return pltpu.make_async_copy(wo_hbm, wo_buf, sems.at[SEM_WO])

    def cp_out(t, c):
        w = D // OC
        return pltpu.make_async_copy(o_buf.at[pl.ds(t * ST, ST), pl.ds(c * w, w)],
                                     o_hbm.at[pl.ds(t * ST, ST), pl.ds(c * w, w)],
                                     sems.at[SEM_OUT + t * OC + c])

    def fold_g(w_buf, dst, g):
        dst[128 * g:128 * (g + 1), :] = (lax.dot_general(
            a_buf[:, 128 * g:128 * (g + 1)], w_buf[:, 128 * g:128 * (g + 1)],
            NT_DIMS, preferred_element_type=F32) * LOG2E).astype(BF16)

    XPT = ST // XR
    GPC = G // WC
    w = D // WC

    cp_wphi().start()
    cp_wk(0).start()
    cp_x(0).start()
    cp_wk(1).start()
    cp_x(1).start()
    cp_wk(2).start()
    cp_wk(3).start()
    for c in range(WC):
        cp_wv(c).start()
    for i in range(XPT, NXC):
        cp_x(i).start()
    cp_wq().start()
    cp_wo().start()

    kvt_acc[...] = jnp.zeros_like(kvt_acc)
    z_acc[...] = jnp.zeros_like(z_acc)

    cp_wphi().wait()
    r = lax.broadcasted_iota(jnp.int32, (128, DH), 0)
    c = lax.broadcasted_iota(jnp.int32, (128, DH), 1)
    perm = ((r % 64) // 2 == c).astype(BF16)
    a = lax.dot_general(perm, wphi_buf[...], NT_DIMS, preferred_element_type=F32)
    r = lax.broadcasted_iota(jnp.int32, (128, D), 0)
    c = lax.broadcasted_iota(jnp.int32, (128, D), 1)
    a_buf[...] = jnp.where((2 * (r // 64) + r % 2) == ((c % 128) // 32), a, 0.0).astype(BF16)

    def fold_c(c):
        for g in range(c * GPC, (c + 1) * GPC):
            fold_g(wk_buf, wfk, g)

    def pt0_piece(r0, r1, s0, s1):
        return lax.dot_general(wfk[r0:r1, :], x_buf[s0:s1, :], NT_DIMS, preferred_element_type=F32)

    cp_wk(0).wait()
    fold_c(0)
    cp_x(0).wait()
    pa = pt0_piece(0, w, 0, XR)
    cp_wk(1).wait()
    fold_c(1)
    pb = pt0_piece(w, 2 * w, 0, XR)
    cp_x(1).wait()
    pc = pt0_piece(0, 2 * w, XR, 2 * XR)
    cp_wk(2).wait()
    fold_c(2)
    pd = pt0_piece(2 * w, 3 * w, 0, ST)
    cp_wk(3).wait()
    fold_c(3)
    for c in range(WC):
        cp_wv(c).wait()
    pe = pt0_piece(3 * w, 4 * w, 0, ST)
    pt0 = jnp.concatenate([jnp.concatenate([jnp.concatenate([pa, pb], axis=0), pc], axis=1), pd, pe], axis=0)
    for c in range(WC):
        wvt[c * w:(c + 1) * w, :] = wv_buf[:, c * w:(c + 1) * w].T

    def p1_body(t, pt, filler):
        xt = x_buf[pl.ds(pl.multiple_of(t * ST, ST), ST), :]
        if pt is None:
            pt = lax.dot_general(wfk[...], xt, NT_DIMS, preferred_element_type=F32)
        vt = lax.dot_general(wvt[...], xt, NT_DIMS, preferred_element_type=F32).astype(BF16)
        for p in range(NP):
            php, phn = _dual_softmax_t(pt[64 * p:64 * (p + 1), :])
            phi = jnp.concatenate([php.reshape(64, ST), phn.reshape(64, ST)], axis=0)
            zp = phi[:, 0:128]
            for j in range(1, ST // 128):
                zp = zp + phi[:, 128 * j:128 * (j + 1)]
            z_acc[p] += zp
            kvt_acc[p] += lax.dot_general(vt[64 * p:64 * (p + 1), :], phi.astype(BF16), NT_DIMS,
                                          preferred_element_type=F32)
        filler()

    def p1_loop(t, carry):
        for i in range(XPT):
            cp_x(t * XPT + i).wait()
        p1_body(t, None, lambda: None)
        return carry

    def fold_q():
        for g in range(G):
            fold_g(wq_buf, wfq, g)

    p1_body(0, pt0, lambda: None)
    lax.fori_loop(1, NTILE - 1, p1_loop, 0)
    for i in range(XPT):
        cp_x((NTILE - 1) * XPT + i).wait()
    cp_wq().wait()
    p1_body(NTILE - 1, None, fold_q)

    r = lax.broadcasted_iota(jnp.int32, (64, 128), 0)
    c = lax.broadcasted_iota(jnp.int32, (64, 128), 1)
    kmask = (c % 2) == (r // 32)
    for p in range(NP):
        lhs2[p] = jnp.where(kmask, kvt_acc[p], 0.0).astype(BF16)
        zc = jnp.sum(z_acc[p], axis=1, keepdims=True)
        zb[p] = jnp.broadcast_to(zc, (128, 128))
    cp_wo().wait()

    def p2_loop(t, carry):
        xt = x_buf[pl.ds(pl.multiple_of(t * ST, ST), ST), :]
        pt = lax.dot_general(wfq[...], xt, NT_DIMS, preferred_element_type=F32)
        parts = []
        for p in range(NP):
            php, phn = _dual_softmax_t(pt[64 * p:64 * (p + 1), :])
            zg = zb[p]
            zp3 = zg[0:64].reshape(8, 8, 128)
            zn3 = zg[64:128].reshape(8, 8, 128)
            dens = []
            for j in range(ST // 128):
                dens.append(jnp.sum(php[:, :, 128 * j:128 * (j + 1)] * zp3, axis=0)
                            + jnp.sum(phn[:, :, 128 * j:128 * (j + 1)] * zn3, axis=0))
            den = _red2(jnp.concatenate(dens, axis=1), jnp.add)
            inv = 1.0 / (den + 1e-6)
            phi = jnp.concatenate([php.reshape(64, ST), phn.reshape(64, ST)], axis=0).astype(BF16)
            num = jnp.dot(lhs2[p], phi, preferred_element_type=F32)
            for hl in range(2):
                parts.append(num[32 * hl:32 * (hl + 1), :] * inv[hl:hl + 1, :])
        ot = jnp.concatenate(parts, axis=0)
        o = ot.T.astype(BF16)
        wo_c = D // OC
        for c in range(OC):
            o_buf[pl.ds(pl.multiple_of(t * ST, ST), ST), c * wo_c:(c + 1) * wo_c] = jnp.dot(
                o, wo_buf[:, c * wo_c:(c + 1) * wo_c], preferred_element_type=F32).astype(BF16)
            cp_out(t, c).start()
        return carry

    lax.fori_loop(0, NTILE, p2_loop, 0)
    for t in range(NTILE):
        for c in range(OC):
            cp_out(t, c).wait()


@jax.jit
def pallas_standalone__linear_kernel_hedgehog__prompt_kernel(
    x: jax.Array,
    wqkv: jax.Array,
    w_phi: jax.Array,
    wo: jax.Array,
):
    x2 = x.reshape(S, D)
    wphi2 = w_phi.reshape(H * DH, DH)
    out = pl.pallas_call(
        _kernel,
        in_specs=[pl.BlockSpec(memory_space=pl.ANY)] * 4,
        out_specs=pl.BlockSpec(memory_space=pl.ANY),
        out_shape=jax.ShapeDtypeStruct((S, D), x.dtype),
        scratch_shapes=[
            pltpu.VMEM((S, D), BF16),
            pltpu.VMEM((D, D), BF16),
            pltpu.VMEM((D, D), BF16),
            pltpu.VMEM((D, D), BF16),
            pltpu.VMEM((D, D), BF16),
            pltpu.VMEM((H * DH, DH), BF16),
            pltpu.VMEM((128, D), BF16),
            pltpu.VMEM((D, D), BF16),
            pltpu.VMEM((D, D), BF16),
            pltpu.VMEM((D, D), BF16),
            pltpu.VMEM((NP, 64, 128), F32),
            pltpu.VMEM((NP, 128, 128), F32),
            pltpu.VMEM((NP, 64, 128), BF16),
            pltpu.VMEM((NP, 128, 128), F32),
            pltpu.VMEM((S, D), BF16),
            pltpu.SemaphoreType.DMA((NSEM,)),
        ],
        compiler_params=pltpu.CompilerParams(
            vmem_limit_bytes=100 * 1024 * 1024,
        ),
    )(x2, wqkv, wphi2, wo)
    return out.reshape(1, S, D)
```
